```python
import os as _os
_os.environ.setdefault("JAX_PLATFORMS", "cpu")
import jax
import jax.numpy as jnp

def _softmax(x, axis=-1):
    return jax.nn.softmax(x, axis=axis)
def _gelu(x):
    return jax.nn.gelu(x, approximate=True)
def _silu(x):
    return jax.nn.silu(x)
def _sigmoid(x):
    return jax.nn.sigmoid(x)
def _layernorm(x, axis=-1, eps=1e-5):
    m = jnp.mean(x, axis=axis, keepdims=True)
    v = jnp.var(x, axis=axis, keepdims=True)
    return (x - m) / jnp.sqrt(v + eps)
def _scatter_add(tgt, idx, src, axis=0):
    return tgt.at[idx].add(src)
def _segment_sum(src, seg, n):
    return jax.ops.segment_sum(src, seg, n)
class _Rng:
    def __init__(self, key):
        self._k = key
    def _next(self):
        self._k, sub = jax.random.split(self._k)
        return sub
    def normal(self, shape):
        return jax.random.normal(self._next(), shape, dtype=jnp.bfloat16)
    def randint(self, lo, hi, shape):
        return jax.random.randint(self._next(), shape, lo, hi, dtype=jnp.int32)
    def uniform(self, shape, lo=0.0, hi=1.0):
        return jax.random.uniform(self._next(), shape, jnp.bfloat16, lo, hi)
    def permutation(self, n):
        return jax.random.permutation(self._next(), n)


kernel_name = 'concat_heads__mha_block_cached__gqa_block_cached__near_ridge'

def setup_inputs():
    _rng = _Rng(jax.random.key(int.from_bytes(__import__("os").urandom(4), "little")))
    _w = (lambda a: (lambda t: t.astype(jnp.bfloat16) if jnp.issubdtype(t.dtype, jnp.floating) else t)(jnp.asarray(a)))
    def _A_setup():
        B, Sq, D = 8, 128, 512
        H, Sk, Dh = 32, 1024, 128
        return {
            "x": _w((lambda *s: _rng.normal(s) * 0.8)(B, Sq, D)),
            "k_cache": _w((lambda *s: _rng.normal(s) * 0.8)(B, H, Sk, Dh)),
            "v_cache": _w((lambda *s: _rng.normal(s) * 0.05)(B, H, Sk, Dh)),
            "wq": _w((lambda *s: _rng.normal(s) * 0.8)(D, H * Dh) * (D ** -0.5)),
            "wo": _w((lambda *s: _rng.normal(s) * 0.05)(H * Dh, D) * ((H * Dh) ** -0.5)),
        }
    _A_in = _A_setup()

    def _B_setup():
        B, Sq, D = 8, 128, 512
        Hq, Hkv, Sk, Dh = 32, 32, 1024, 128
        assert Hq % Hkv == 0, (Hq, Hkv)
        return {
            "x": _w((lambda *s: _rng.normal(s) * 0.8)(B, Sq, D)),
            "k_cache": _w((lambda *s: _rng.normal(s) * 0.8)(B, Hkv, Sk, Dh)),
            "v_cache": _w((lambda *s: _rng.normal(s) * 0.05)(B, Hkv, Sk, Dh)),
            "wq": _w((lambda *s: _rng.normal(s) * 0.8)(D, Hq * Dh) * (D ** -0.5)),
            "wo": _w((lambda *s: _rng.normal(s) * 0.05)(Hq * Dh, D) * ((Hq * Dh) ** -0.5)),
        }
    _B_in = _B_setup()

    return {
        "A_x": _A_in["x"],
        "A_k_cache": _A_in["k_cache"],
        "A_v_cache": _A_in["v_cache"],
        "A_wq": _A_in["wq"],
        "A_wo": _A_in["wo"],
        "B_x": _B_in["x"],
        "B_k_cache": _B_in["k_cache"],
        "B_v_cache": _B_in["v_cache"],
        "B_wq": _B_in["wq"],
        "B_wo": _B_in["wo"],
    }

def reference(A_x, A_k_cache, A_v_cache, A_wq, A_wo, B_x, B_k_cache, B_v_cache, B_wq, B_wo):
    def _A_ref(x, k_cache, v_cache, wq, wo):
        B, Sq, D = x.shape
        H, Dh = 32, 128
        q = (lambda x, *d: x.transpose(*d))((x @ wq).reshape(B, Sq, H, Dh), 0, 2, 1, 3)
        scores = jnp.einsum("bhqd,bhkd->bhqk", q, k_cache) * (Dh ** -0.5)
        p = _softmax(scores, axis=-1)
        o = jnp.einsum("bhqk,bhkd->bhqd", p, v_cache)
        return (lambda x, *d: x.transpose(*d))(o, 0, 2, 1, 3).reshape(B, Sq, H * Dh) @ wo

    def _B_ref(x, k_cache, v_cache, wq, wo):
        B, Sq, D = x.shape
        Hq, Dh = 32, 128
        Hkv = k_cache.shape[1]
        rep = Hq // Hkv
        q = (lambda x, *d: x.transpose(*d))((x @ wq).reshape(B, Sq, Hq, Dh), 0, 2, 1, 3)
        k = jnp.repeat(k_cache, rep, axis=1)
        v = jnp.repeat(v_cache, rep, axis=1)
        scores = jnp.einsum("bhqd,bhkd->bhqk", q, k) * (Dh ** -0.5)
        p = _softmax(scores, axis=-1)
        o = jnp.einsum("bhqk,bhkd->bhqd", p, v)
        return (lambda x, *d: x.transpose(*d))(o, 0, 2, 1, 3).reshape(B, Sq, Hq * Dh) @ wo

    a = _A_ref(A_x, A_k_cache, A_v_cache, A_wq, A_wo)
    b = _B_ref(B_x, B_k_cache, B_v_cache, B_wq, B_wo)
    return jnp.concatenate([a, b], axis=-1)
```

```python
import functools
import math
import jax
import jax.numpy as jnp
import jax.experimental.pallas as pl
import jax.experimental.pallas.tpu as pltpu

NB = 4
NO_DMA = False

_NT = (((1,), (1,)), ((), ()))


def _kernel(xa, ka, va, wqa, woa, xb, kb, vb, wqb, wob, out_hbm,
            xbuf, wqbuf, wobuf, kbuf, vbuf, s0, s1, m0, m1, p0, p1, r0, r1, acc, obuf,
            wsem, ksem, vsem, osem, *, n_pair_per_prob, pairs_per_batch, qscale):
    NP = 2 * n_pair_per_prob
    D = xbuf.shape[-1]

    def kv_copy(which, j, prob):
        src = ((ka, kb), (va, vb))[which][prob]
        buf = (kbuf, vbuf)[which]
        sem = (ksem, vsem)[which]
        slot = j % NB
        return pltpu.make_async_copy(src.at[j - prob * n_pair_per_prob], buf.at[slot], sem.at[slot])

    def start_kv(which, j):
        if isinstance(j, int):
            if j < NP:
                kv_copy(which, j, j // n_pair_per_prob).start()
            return
        @pl.when(j < n_pair_per_prob)
        def _():
            kv_copy(which, j, 0).start()
        @pl.when(jnp.logical_and(j >= n_pair_per_prob, j < NP))
        def _():
            kv_copy(which, j, 1).start()

    def wait_kv(which, j):
        buf = (kbuf, vbuf)[which]
        sem = (ksem, vsem)[which]
        slot = j % NB
        pltpu.make_async_copy(buf.at[slot], buf.at[slot], sem.at[slot]).wait()

    w_copies = [
        pltpu.make_async_copy(xa, xbuf.at[0], wsem.at[0]),
        pltpu.make_async_copy(wqa, wqbuf.at[0], wsem.at[1]),
        pltpu.make_async_copy(woa, wobuf.at[0], wsem.at[2]),
        pltpu.make_async_copy(xb, xbuf.at[1], wsem.at[3]),
        pltpu.make_async_copy(wqb, wqbuf.at[1], wsem.at[4]),
        pltpu.make_async_copy(wob, wobuf.at[1], wsem.at[5]),
    ]

    def idx(j):
        p = j // n_pair_per_prob
        b = (j // pairs_per_batch) % (n_pair_per_prob // pairs_per_batch)
        hp = j % pairs_per_batch
        return p, b, hp

    def stage_A(j):
        p, b, hp = idx(j)
        c0 = pl.multiple_of(hp * 256, 256)
        q = jnp.dot(xbuf[p, b], wqbuf[p, :, pl.ds(c0, 256)], preferred_element_type=jnp.float32)
        return (q * qscale).astype(jnp.bfloat16)

    def stage_B(q, j, i, s_ref, m_ref):
        k = kbuf[j % NB, i]
        s = jax.lax.dot_general(q, k, _NT, preferred_element_type=jnp.float32)
        s_ref[...] = s
        m_ref[...] = jnp.broadcast_to(jnp.max(s, axis=-1, keepdims=True), m_ref.shape)

    def stage_C(s_ref, m_ref, p_ref, r_ref):
        m = m_ref[...]
        n = s_ref.shape[1] // 128
        lsum = None
        for c in range(n):
            pc = jnp.exp2(s_ref[:, c * 128:(c + 1) * 128] - m)
            lsum = pc if lsum is None else lsum + pc
            p_ref[:, c * 128:(c + 1) * 128] = pc.astype(jnp.bfloat16)
        l = jnp.sum(lsum, axis=-1, keepdims=True)
        r_ref[...] = jnp.broadcast_to(1.0 / l, r_ref.shape)

    def stage_D(j, i, p_ref, r_ref):
        v = vbuf[j % NB, i]
        o = jnp.dot(p_ref[...], v, preferred_element_type=jnp.float32)
        return (o * r_ref[...]).astype(jnp.bfloat16)

    def stage_E(j, o0, o1):
        p, b, hp = idx(j)
        c0 = pl.multiple_of(hp * 256, 256)
        o = jnp.concatenate([o0, o1], axis=-1)
        acc[...] += jnp.dot(o, wobuf[p, pl.ds(c0, 256), :], preferred_element_type=jnp.float32)

    def out_copy(p, b):
        return pltpu.make_async_copy(obuf, out_hbm.at[b, :, pl.ds(pl.multiple_of(p * D, D), D)], osem.at[0])

    def flush_out(j, first_possible):
        p, b, hp = idx(j)
        if first_possible:
            @pl.when(j >= pairs_per_batch)
            def _():
                out_copy(p, b).wait()
        else:
            out_copy(p, b).wait()
        obuf[...] = acc[...].astype(obuf.dtype)
        acc[...] = jnp.zeros_like(acc)
        out_copy(p, b).start()

    def body(j, doAB, doDE):
        if doAB:
            q = stage_A(j)
        if doDE:
            stage_C(s1, m1, p1, r1)
            o0 = stage_D(j - 1, 0, p0, r0)
        if doAB:
            stage_B(q[:, :128], j, 0, s0, m0)
        if doDE:
            o1 = stage_D(j - 1, 1, p1, r1)
        if doAB:
            stage_C(s0, m0, p0, r0)
            stage_B(q[:, 128:], j, 1, s1, m1)
        if doDE:
            stage_E(j - 1, o0, o1)

    w_copies[0].start()
    w_copies[1].start()
    start_kv(0, 0)
    start_kv(1, 0)
    start_kv(0, 1)
    w_copies[2].start()
    for t in range(2, NB):
        start_kv(0, t)
        start_kv(1, t - 1)
    for c in w_copies[3:]:
        c.start()
    acc[...] = jnp.zeros_like(acc)
    w_copies[0].wait()
    w_copies[1].wait()
    wait_kv(0, 0)
    body(0, True, False)
    w_copies[2].wait()

    def loop(j, carry):
        if not NO_DMA:
            start_kv(0, j - 1 + NB)
            start_kv(1, j - 2 + NB)
        @pl.when(j == n_pair_per_prob)
        def _():
            for c in w_copies[3:]:
                c.wait()
        if NO_DMA:
            @pl.when(j < NB)
            def _():
                wait_kv(0, j)
            @pl.when(j < NB)
            def _():
                wait_kv(1, j - 1)
        else:
            wait_kv(0, j)
            wait_kv(1, j - 1)
        body(j, True, True)
        @pl.when((j - 1) % pairs_per_batch == pairs_per_batch - 1)
        def _():
            flush_out(j - 1, True)
        return carry

    jax.lax.fori_loop(1, NP, loop, 0)

    if not NO_DMA:
        wait_kv(1, NP - 1)
    body(NP, False, True)
    flush_out(NP - 1, False)
    p, b, _ = idx(NP - 1)
    out_copy(p, b).wait()


@jax.jit
def pallas_concat_heads__mha_block_cached__gqa_block_cached__near_ridge_kernel(
    A_x, A_k_cache, A_v_cache, A_wq, A_wo, B_x, B_k_cache, B_v_cache, B_wq, B_wo):
    B, Sq, D = A_x.shape
    _, H, Sk, Dh = A_k_cache.shape
    npp = B * H // 2
    r = lambda a: a.reshape(npp, 2, Sk, Dh)
    qscale = (Dh ** -0.5) * math.log2(math.e)
    kern = functools.partial(_kernel, n_pair_per_prob=npp, pairs_per_batch=H // 2, qscale=qscale)
    bf = jnp.bfloat16
    f32 = jnp.float32
    return pl.pallas_call(
        kern,
        in_specs=[pl.BlockSpec(memory_space=pl.ANY)] * 10,
        out_specs=pl.BlockSpec(memory_space=pl.ANY),
        out_shape=jax.ShapeDtypeStruct((B, Sq, 2 * D), A_x.dtype),
        scratch_shapes=[
            pltpu.VMEM((2, B, Sq, D), bf),
            pltpu.VMEM((2, D, H * Dh), bf),
            pltpu.VMEM((2, H * Dh, D), bf),
            pltpu.VMEM((NB, 2, Sk, Dh), bf),
            pltpu.VMEM((NB, 2, Sk, Dh), bf),
            pltpu.VMEM((Sq, Sk), f32), pltpu.VMEM((Sq, Sk), f32),
            pltpu.VMEM((Sq, 128), f32), pltpu.VMEM((Sq, 128), f32),
            pltpu.VMEM((Sq, Sk), bf), pltpu.VMEM((Sq, Sk), bf),
            pltpu.VMEM((Sq, 128), f32), pltpu.VMEM((Sq, 128), f32),
            pltpu.VMEM((Sq, D), f32),
            pltpu.VMEM((Sq, D), bf),
            pltpu.SemaphoreType.DMA((6,)),
            pltpu.SemaphoreType.DMA((NB,)),
            pltpu.SemaphoreType.DMA((NB,)),
            pltpu.SemaphoreType.DMA((1,)),
        ],
        compiler_params=pltpu.CompilerParams(vmem_limit_bytes=100 * 1024 * 1024),
    )(A_x, r(A_k_cache), r(A_v_cache), A_wq, A_wo, B_x, r(B_k_cache), r(B_v_cache), B_wq, B_wo)
```

```python
import functools
import math
import jax
import jax.numpy as jnp
from jax import lax
import jax.experimental.pallas as pl
import jax.experimental.pallas.tpu as pltpu

NB = 4
NO_DMA = False
PIECE = 128
NPTS = 8
PRIO = (0, 1, 1, 1)
KV_U32 = True
P_U32 = True
NO_COMPUTE = False
NO_TAIL = False
NO_HEAD = False

_NT = (((1,), (1,)), ((), ()))

def _slot(j):
    if isinstance(j, int):
        return j % NB
    if NB & (NB - 1) == 0:
        return j & (NB - 1)
    return lax.rem(j, NB)


def _kernel(xa, ka, va, wqa, woa, xb, kb, vb, wqb, wob, out_hbm,
            xbuf, wqbuf, wobuf, kbuf, vbuf, s0, s1, m0, m1, p0, p1, r0, r1, acc, obuf,
            wsem, ksem, vsem, osem, *, n_units, n_heads, qscale):
    N = n_units
    D = xbuf.shape[-1]
    Sk = ka.shape[1]
    hshift = n_heads.bit_length() - 1
    pk = 2 if KV_U32 else 1

    if KV_U32:
        srcs = [r.bitcast(jnp.uint32) for r in (ka, va, kb, vb)]
    else:
        srcs = [ka, va, kb, vb]

    def piece_copy(s, j, off, rows):
        buf = (kbuf, vbuf)[s % 2]
        sem = (ksem, vsem)[s % 2]
        slot = _slot(j)
        return pltpu.make_async_copy(
            srcs[s].at[j, pl.ds(off // pk, rows // pk)],
            buf.at[slot, s // 2, pl.ds(off // pk, rows // pk)],
            sem.at[slot])

    npieces = 4 * Sk // PIECE
    per = npieces // NPTS
    sched = [[] for _ in range(NPTS)]
    for i in range(npieces):
        sched[i // per].append((i % 4, (i // 4) * PIECE, PRIO[i % len(PRIO)]))

    def issue(pt, jk, jv, guard):
        def go(which):
            for (s, off, pr) in sched[pt]:
                if s % 2 == which:
                    piece_copy(s, (jk, jv)[which], off, PIECE).start(priority=pr)
        if guard is None:
            for (s, off, pr) in sched[pt]:
                j = (jk, jv)[s % 2]
                if j is not None:
                    piece_copy(s, j, off, PIECE).start(priority=pr)
        else:
            raise NotImplementedError

    def wait_kv(which, j):
        buf = (kbuf, vbuf)[which]
        sem = (ksem, vsem)[which]
        slot = _slot(j)
        pltpu.make_async_copy(buf.at[slot], buf.at[slot], sem.at[slot]).wait()

    w_copies = [
        pltpu.make_async_copy(xa, xbuf.at[0], wsem.at[0]),
        pltpu.make_async_copy(wqa, wqbuf.at[0], wsem.at[1]),
        pltpu.make_async_copy(xb, xbuf.at[1], wsem.at[2]),
        pltpu.make_async_copy(wqb, wqbuf.at[1], wsem.at[3]),
        pltpu.make_async_copy(woa, wobuf.at[0], wsem.at[4]),
        pltpu.make_async_copy(wob, wobuf.at[1], wsem.at[5]),
    ]

    def bh(j):
        return j >> hshift, j & (n_heads - 1)

    def load_kv(buf, j, p):
        v = buf[_slot(j), p]
        if KV_U32:
            v = pltpu.bitcast(v, jnp.bfloat16)
        return v

    def stage_A(j, p):
        b, h = bh(j)
        c0 = pl.multiple_of(h * 128, 128)
        q = jnp.dot(xbuf[p, b], wqbuf[p, :, pl.ds(c0, 128)], preferred_element_type=jnp.float32)
        return (q * qscale).astype(jnp.bfloat16)

    def stage_B(q, j, p, s_ref, m_ref):
        k = load_kv(kbuf, j, p)
        s = lax.dot_general(q, k, _NT, preferred_element_type=jnp.float32)
        s_ref[...] = s
        m_ref[...] = jnp.broadcast_to(jnp.max(s, axis=-1, keepdims=True), m_ref.shape)

    def stage_C(s_ref, m_ref, p_ref, r_ref):
        m = m_ref[...]
        n = s_ref.shape[1] // 128
        lsum = None
        for c in range(n):
            pc = jnp.exp2(s_ref[:, c * 128:(c + 1) * 128] - m)
            lsum = pc if lsum is None else lsum + pc
            pb = pc.astype(jnp.bfloat16)
            if P_U32:
                pb = pltpu.bitcast(pb, jnp.uint32)
            p_ref[:, c * 128:(c + 1) * 128] = pb
        l = jnp.sum(lsum, axis=-1, keepdims=True)
        r_ref[...] = jnp.broadcast_to(1.0 / l, r_ref.shape)

    def stage_D(j, p, p_ref, r_ref):
        v = load_kv(vbuf, j, p)
        pp = p_ref[...]
        if P_U32:
            pp = pltpu.bitcast(pp, jnp.bfloat16)
        o = jnp.dot(pp, v, preferred_element_type=jnp.float32)
        return (o * r_ref[...]).astype(jnp.bfloat16)

    def stage_E(j, p, o):
        b, h = bh(j)
        c0 = pl.multiple_of(h * 128, 128)
        acc[:, p * D:(p + 1) * D] += jnp.dot(o, wobuf[p, pl.ds(c0, 128), :], preferred_element_type=jnp.float32)

    def out_copy(b):
        return pltpu.make_async_copy(obuf, out_hbm.at[b], osem.at[0])

    def flush_out(j, first_possible):
        b, h = bh(j)
        if first_possible:
            @pl.when(b > 0)
            def _():
                out_copy(b).wait()
        else:
            out_copy(b).wait()
        obuf[...] = acc[...].astype(obuf.dtype)
        acc[...] = jnp.zeros_like(acc)
        out_copy(b).start()

    def body(j, doAB, doDE, jk=None, jv=None):
        pts = iter(range(NPTS))
        def pt():
            if jk is not None or jv is not None:
                t = next(pts, None)
                if t is not None:
                    issue(t, jk, jv, None)
        if NO_COMPUTE or (NO_TAIL and jk is None and jv is None and doDE) or (NO_HEAD and jk is not None):
            doAB = doDE = False
        pt()
        if doAB:
            qa = stage_A(j, 0)
            qb = stage_A(j, 1)
        pt()
        if doDE:
            stage_C(s1, m1, p1, r1)
            pt()
            o0 = stage_D(j - 1, 0, p0, r0)
        pt()
        if doAB:
            stage_B(qa, j, 0, s0, m0)
        pt()
        if doDE:
            o1 = stage_D(j - 1, 1, p1, r1)
        pt()
        if doAB:
            stage_C(s0, m0, p0, r0)
            pt()
            stage_B(qb, j, 1, s1, m1)
        pt()
        if doDE:
            stage_E(j - 1, 0, o0)
            stage_E(j - 1, 1, o1)
        for _ in range(NPTS):
            pt()

    def issue_all(jk, jv):
        for t in range(NPTS):
            issue(t, jk, jv, None)

    for c in w_copies[:4]:
        c.start()
    issue_all(0, None)
    issue_all(1, 0)
    for c in w_copies[4:]:
        c.start()
    for t in range(2, NB):
        issue_all(t, t - 1)
    acc[...] = jnp.zeros_like(acc)
    for c in w_copies[:4]:
        c.wait()
    wait_kv(0, 0)
    body(0, True, False)
    for c in w_copies[4:]:
        c.wait()

    def make_loop(dok, dov):
        def loop(j, carry):
            if NO_DMA:
                @pl.when(j < NB)
                def _():
                    wait_kv(0, j)
                    wait_kv(1, j - 1)
                body(j, True, True)
            else:
                wait_kv(0, j)
                wait_kv(1, j - 1)
                body(j, True, True, j - 1 + NB if dok else None, j - 2 + NB if dov else None)
            @pl.when(((j - 1) & (n_heads - 1)) == n_heads - 1)
            def _():
                flush_out(j - 1, True)
            return carry
        return loop

    lax.fori_loop(1, N - NB + 1, make_loop(True, True), 0)
    if not NO_DMA:
        issue_all(None, N - 1)
    lax.fori_loop(N - NB + 1, N, make_loop(False, False), 0)

    if not NO_DMA:
        wait_kv(1, N - 1)
    body(N, False, True)
    flush_out(N - 1, False)
    out_copy((N - 1) >> hshift).wait()


@jax.jit
def pallas_concat_heads__mha_block_cached__gqa_block_cached__near_ridge_kernel(
    A_x, A_k_cache, A_v_cache, A_wq, A_wo, B_x, B_k_cache, B_v_cache, B_wq, B_wo):
    B, Sq, D = A_x.shape
    _, H, Sk, Dh = A_k_cache.shape
    n = B * H
    r = lambda a: a.reshape(n, Sk, Dh)
    qscale = (Dh ** -0.5) * math.log2(math.e)
    kern = functools.partial(_kernel, n_units=n, n_heads=H, qscale=qscale)
    bf = jnp.bfloat16
    f32 = jnp.float32
    u32 = jnp.uint32
    kvs = pltpu.VMEM((NB, 2, Sk // 2, Dh), u32) if KV_U32 else pltpu.VMEM((NB, 2, Sk, Dh), bf)
    ps = pltpu.VMEM((Sq // 2, Sk), u32) if P_U32 else pltpu.VMEM((Sq, Sk), bf)
    return pl.pallas_call(
        kern,
        in_specs=[pl.BlockSpec(memory_space=pl.ANY)] * 10,
        out_specs=pl.BlockSpec(memory_space=pl.ANY),
        out_shape=jax.ShapeDtypeStruct((B, Sq, 2 * D), A_x.dtype),
        scratch_shapes=[
            pltpu.VMEM((2, B, Sq, D), bf),
            pltpu.VMEM((2, D, H * Dh), bf),
            pltpu.VMEM((2, H * Dh, D), bf),
            kvs, kvs,
            pltpu.VMEM((Sq, Sk), f32), pltpu.VMEM((Sq, Sk), f32),
            pltpu.VMEM((Sq, 128), f32), pltpu.VMEM((Sq, 128), f32),
            ps, ps,
            pltpu.VMEM((Sq, 128), f32), pltpu.VMEM((Sq, 128), f32),
            pltpu.VMEM((Sq, 2 * D), f32),
            pltpu.VMEM((Sq, 2 * D), bf),
            pltpu.SemaphoreType.DMA((6,)),
            pltpu.SemaphoreType.DMA((NB,)),
            pltpu.SemaphoreType.DMA((NB,)),
            pltpu.SemaphoreType.DMA((1,)),
        ],
        compiler_params=pltpu.CompilerParams(vmem_limit_bytes=100 * 1024 * 1024, disable_bounds_checks=True),
    )(A_x, r(A_k_cache), r(A_v_cache), A_wq, A_wo, B_x, r(B_k_cache), r(B_v_cache), B_wq, B_wo)
```

```python
import functools
import math
import jax
import jax.numpy as jnp
from jax import lax
import jax.experimental.pallas as pl
import jax.experimental.pallas.tpu as pltpu

NB = 8
L = 3
PIECE = 64
PRIO = (0, 1, 1, 1, 0, 1, 1, 1)
NO_COMPUTE = False
WPRIO = (0, 1, 1, 1)
GRP = 2
TSWITCH = 8

_NT = (((1,), (1,)), ((), ()))


def _kernel(xa, ka, va, wqa, woa, xb, kb, vb, wqb, wob, out_hbm,
            xbuf, wqbuf, wobuf, kvbuf, s0, s1, m0, m1, p0, p1, r0, r1, acc, obuf,
            wsem, kvsem, osem, *, n_units, n_heads, qscale):
    N = n_units
    D = xbuf.shape[-1]
    Sk = ka.shape[1]
    hshift = n_heads.bit_length() - 1
    NPC = Sk // PIECE
    assert L <= NB - 2

    srcs = [ka, va, kb, vb]

    def slot_of(t):
        return t & (NB - 1)

    def unit_of(t):
        return (t & 1) * (N // 2) + (t >> 1)

    def piece_copy(s, t, off):
        slot = slot_of(t)
        return pltpu.make_async_copy(
            srcs[s].at[unit_of(t), pl.ds(off, PIECE)],
            kvbuf.at[s % 2, slot, s // 2, pl.ds(off, PIECE)],
            kvsem.at[s % 2, slot])

    def start_piece(s, need_t, off, pr):
        t = need_t - (s % 2)
        if isinstance(t, int):
            if 0 <= t < N:
                piece_copy(s, t, off).start(priority=pr)
        else:
            @pl.when(t < N)
            def _():
                piece_copy(s, t, pl.multiple_of(off, PIECE)).start(priority=pr)

    def issue(pt, t):
        i, second = pt // 2, pt % 2
        inter = t < N - TSWITCH
        need = jnp.where(inter, (t & ~1) + L + second, t + L)
        off = jnp.where(inter, (t & 1) * (Sk // 2) + i * PIECE, pt * PIECE)
        for s in range(4):
            start_piece(s, need, off, PRIO[4 * second + s])

    def wait_kv(which, t):
        slot = slot_of(t)
        pltpu.make_async_copy(kvbuf.at[which, slot], kvbuf.at[which, slot], kvsem.at[which, slot]).wait()

    w_copies = [
        pltpu.make_async_copy(xa, xbuf.at[0], wsem.at[0]),
        pltpu.make_async_copy(wqa, wqbuf.at[0], wsem.at[1]),
        pltpu.make_async_copy(xb, xbuf.at[1], wsem.at[2]),
        pltpu.make_async_copy(wqb, wqbuf.at[1], wsem.at[3]),
        pltpu.make_async_copy(woa, wobuf.at[0], wsem.at[4]),
        pltpu.make_async_copy(wob, wobuf.at[1], wsem.at[5]),
    ]

    def bh(t):
        u = unit_of(t)
        return u >> hshift, u & (n_heads - 1)

    def stage_A(t, p):
        b, h = bh(t)
        c0 = pl.multiple_of(h * 128, 128)
        q = jnp.dot(xbuf[p, b], wqbuf[p, :, pl.ds(c0, 128)], preferred_element_type=jnp.float32)
        return (q * qscale).astype(jnp.bfloat16)

    def stage_B(q, t, p, s_ref, m_ref):
        k = kvbuf[0, slot_of(t), p]
        s = lax.dot_general(q, k, _NT, preferred_element_type=jnp.float32)
        s_ref[...] = s
        m_ref[...] = jnp.broadcast_to(jnp.max(s, axis=-1, keepdims=True), m_ref.shape)

    def stage_C(s_ref, m_ref, p_ref, r_ref):
        m = m_ref[...]
        n = s_ref.shape[1] // 128
        lsum = None
        for c in range(n):
            pc = jnp.exp2(s_ref[:, c * 128:(c + 1) * 128] - m)
            lsum = pc if lsum is None else lsum + pc
            p_ref[:, c * 128:(c + 1) * 128] = pltpu.bitcast(pc.astype(jnp.bfloat16), jnp.uint32)
        l = jnp.sum(lsum, axis=-1, keepdims=True)
        r_ref[...] = jnp.broadcast_to(1.0 / l, r_ref.shape)

    def stage_D(t, p, p_ref, r_ref):
        v = kvbuf[1, slot_of(t), p]
        pp = pltpu.bitcast(p_ref[...], jnp.bfloat16)
        o = jnp.dot(pp, v, preferred_element_type=jnp.float32)
        return (o * r_ref[...]).astype(jnp.bfloat16)

    def stage_E(t, p, o):
        b, h = bh(t)
        c0 = pl.multiple_of(h * 128, 128)
        acc[t & 1, :, p * D:(p + 1) * D] += jnp.dot(o, wobuf[p, pl.ds(c0, 128), :], preferred_element_type=jnp.float32)

    def out_copy(g, b):
        return pltpu.make_async_copy(obuf.at[g], out_hbm.at[b], osem.at[g])

    def flush_out(t, first_possible):
        b, h = bh(t)
        g = t & 1
        if first_possible:
            @pl.when(t >= 2 * n_heads)
            def _():
                out_copy(g, b).wait()
        else:
            out_copy(g, b).wait()
        obuf[g] = acc[g].astype(obuf.dtype)
        acc[g] = jnp.zeros(acc.shape[1:], acc.dtype)
        out_copy(g, b).start()

    def body(t, doAB, doDE, do_issue):
        if NO_COMPUTE:
            doAB = doDE = False
        pts = iter(range(NPC))
        def pt():
            if do_issue:
                for _ in range(GRP):
                    i = next(pts, None)
                    if i is not None:
                        issue(i, t)
        pt()
        if doAB:
            qa = stage_A(t, 0)
            qb = stage_A(t, 1)
        pt()
        if doDE:
            stage_C(s1, m1, p1, r1)
            pt()
            o0 = stage_D(t - 1, 0, p0, r0)
        pt()
        if doAB:
            stage_B(qa, t, 0, s0, m0)
        pt()
        if doDE:
            o1 = stage_D(t - 1, 1, p1, r1)
        pt()
        if doAB:
            stage_C(s0, m0, p0, r0)
            pt()
            stage_B(qb, t, 1, s1, m1)
        pt()
        if doDE:
            stage_E(t - 1, 0, o0)
            stage_E(t - 1, 1, o1)
        for _ in range(NPC):
            pt()

    HD = wqbuf.shape[-1]
    QC = HD // 2
    OR = 32
    nwp = (D // 8) * 2
    assert nwp == HD // OR
    XR = 32
    nxp = xbuf.shape[1] * xbuf.shape[2] // XR
    xpb = xbuf.shape[2] // XR

    def wloop(i, c):
        r8 = pl.multiple_of((i >> 1) * 8, 8)
        c0 = pl.multiple_of((i & 1) * QC, QC)
        r32 = pl.multiple_of(i * OR, OR)
        for p, (wq, wo) in enumerate(((wqa, woa), (wqb, wob))):
            pltpu.make_async_copy(wq.at[pl.ds(r8, 8), pl.ds(c0, QC)], wqbuf.at[p, pl.ds(r8, 8), pl.ds(c0, QC)],
                                  wsem.at[1 + 2 * p]).start(priority=WPRIO[2 * p])
            pltpu.make_async_copy(wo.at[pl.ds(r32, OR)], wobuf.at[p, pl.ds(r32, OR)],
                                  wsem.at[4 + p]).start(priority=WPRIO[2 * p + 1])
        return c

    def xloop(i, c):
        b = i // xpb
        r = pl.multiple_of((i % xpb) * XR, XR)
        for p, x in enumerate((xa, xb)):
            pltpu.make_async_copy(x.at[b, pl.ds(r, XR)], xbuf.at[p, b, pl.ds(r, XR)], wsem.at[2 * p]).start(priority=p)
        return c

    lax.fori_loop(0, nxp, xloop, 0)
    lax.fori_loop(0, nwp, wloop, 0)
    for need in range(L):
        for pc in range(NPC):
            for s in range(4):
                start_piece(s, need, pc * PIECE, PRIO[s])
    acc[...] = jnp.zeros_like(acc)
    for c in w_copies[:4]:
        c.wait()
    wait_kv(0, 0)
    body(jnp.int32(0), True, False, True)
    for c in w_copies[4:]:
        c.wait()

    def loop(t, carry):
        wait_kv(0, t)
        wait_kv(1, t - 1)
        body(t, True, True, True)
        @pl.when((unit_of(t - 1) & (n_heads - 1)) == n_heads - 1)
        def _():
            flush_out(t - 1, True)
        return carry

    lax.fori_loop(1, N, loop, 0)

    wait_kv(1, N - 1)
    body(N, False, True, False)
    flush_out(N - 1, False)
    out_copy(0, bh(N - 2)[0]).wait()
    out_copy(1, bh(N - 1)[0]).wait()


@jax.jit
def pallas_concat_heads__mha_block_cached__gqa_block_cached__near_ridge_kernel(
    A_x, A_k_cache, A_v_cache, A_wq, A_wo, B_x, B_k_cache, B_v_cache, B_wq, B_wo):
    B, Sq, D = A_x.shape
    _, H, Sk, Dh = A_k_cache.shape
    n = B * H
    r = lambda a: a.reshape(n, Sk, Dh)
    qscale = (Dh ** -0.5) * math.log2(math.e)
    kern = functools.partial(_kernel, n_units=n, n_heads=H, qscale=qscale)
    bf = jnp.bfloat16
    f32 = jnp.float32
    u32 = jnp.uint32
    ps = pltpu.VMEM((Sq // 2, Sk), u32)
    return pl.pallas_call(
        kern,
        in_specs=[pl.BlockSpec(memory_space=pl.ANY)] * 10,
        out_specs=pl.BlockSpec(memory_space=pl.ANY),
        out_shape=jax.ShapeDtypeStruct((B, Sq, 2 * D), A_x.dtype),
        scratch_shapes=[
            pltpu.VMEM((2, B, Sq, D), bf),
            pltpu.VMEM((2, D, H * Dh), bf),
            pltpu.VMEM((2, H * Dh, D), bf),
            pltpu.VMEM((2, NB, 2, Sk, Dh), bf),
            pltpu.VMEM((Sq, Sk), f32), pltpu.VMEM((Sq, Sk), f32),
            pltpu.VMEM((Sq, 128), f32), pltpu.VMEM((Sq, 128), f32),
            ps, ps,
            pltpu.VMEM((Sq, 128), f32), pltpu.VMEM((Sq, 128), f32),
            pltpu.VMEM((2, Sq, 2 * D), f32),
            pltpu.VMEM((2, Sq, 2 * D), bf),
            pltpu.SemaphoreType.DMA((6,)),
            pltpu.SemaphoreType.DMA((2, NB)),
            pltpu.SemaphoreType.DMA((2,)),
        ],
        compiler_params=pltpu.CompilerParams(vmem_limit_bytes=100 * 1024 * 1024, disable_bounds_checks=True),
    )(A_x, r(A_k_cache), r(A_v_cache), A_wq, A_wo, B_x, r(B_k_cache), r(B_v_cache), B_wq, B_wo)
```

```python
import functools
import math
import jax
import jax.numpy as jnp
from jax import lax
import jax.experimental.pallas as pl
import jax.experimental.pallas.tpu as pltpu

NB = 8
L = 3
PIECE = 64
PRIO = (0, 1, 1, 1, 0, 1, 1, 1)
NO_COMPUTE = False
WPRIO = (0, 1, 1, 1)
GRP = 2
R1 = 16
NEARLY = 0
OPRIO = 1
TDEF = (3, 3, 3, 3, 3, 3)
ROT = (0, 0, 0, 0)
R2 = 0
TSWITCH = 8

_NT = (((1,), (1,)), ((), ()))


def _kernel(xa, ka, va, wqa, woa, xb, kb, vb, wqb, wob, out_hbm,
            xbuf, wqbuf, wobuf, kvbuf, s0, s1, m0, m1, p0, p1, r0, r1, acc, obuf,
            wsem, kvsem, osem, *, n_units, n_heads, qscale):
    N = n_units
    D = xbuf.shape[-1]
    Sk = ka.shape[1]
    hshift = n_heads.bit_length() - 1
    NPC = Sk // PIECE
    assert L <= NB - 2

    srcs = [ka, va, kb, vb]

    def slot_of(t):
        return t & (NB - 1)

    def unit_of(t, p):
        g, j = t & 1, t >> 1
        return g * (N // 2) + (j & ~(n_heads - 1)) + ((j + g * R1 + p * R2) & (n_heads - 1))

    def piece_copy(s, t, off):
        slot = slot_of(t)
        return pltpu.make_async_copy(
            srcs[s].at[unit_of(t, s // 2), pl.ds(off, PIECE)],
            kvbuf.at[s % 2, slot, s // 2, pl.ds(off, PIECE)],
            kvsem.at[s % 2, slot])

    def start_piece(s, need_t, off, pr):
        t = need_t - (s % 2)
        off = (off + ROT[s]) & (Sk - 1)
        if isinstance(t, int):
            if 0 <= t < N:
                piece_copy(s, t, off).start(priority=pr)
        else:
            @pl.when(t < N)
            def _():
                piece_copy(s, t, pl.multiple_of(off, PIECE)).start(priority=pr)

    def issue(pt, t):
        i, second = pt // 2, pt % 2
        inter = t < N - TSWITCH
        need = jnp.where(inter, (t & ~1) + L + second, t + L)
        off = jnp.where(inter, (t & 1) * (Sk // 2) + i * PIECE, pt * PIECE)
        for s in range(4):
            start_piece(s, need, off, PRIO[4 * second + s])

    def wait_kv(which, t):
        slot = slot_of(t)
        pltpu.make_async_copy(kvbuf.at[which, slot], kvbuf.at[which, slot], kvsem.at[which, slot]).wait()

    w_copies = [
        pltpu.make_async_copy(xa, xbuf.at[0], wsem.at[0]),
        pltpu.make_async_copy(wqa, wqbuf.at[0], wsem.at[1]),
        pltpu.make_async_copy(xb, xbuf.at[1], wsem.at[2]),
        pltpu.make_async_copy(wqb, wqbuf.at[1], wsem.at[3]),
        pltpu.make_async_copy(woa, wobuf.at[0], wsem.at[4]),
        pltpu.make_async_copy(wob, wobuf.at[1], wsem.at[5]),
    ]

    def bh(t, p=0):
        u = unit_of(t, p)
        return u >> hshift, u & (n_heads - 1)

    def stage_A(t, p):
        b, h = bh(t, p)
        c0 = pl.multiple_of(h * 128, 128)
        q = jnp.dot(xbuf[p, b], wqbuf[p, :, pl.ds(c0, 128)], preferred_element_type=jnp.float32)
        return (q * qscale).astype(jnp.bfloat16)

    def stage_B(q, t, p, s_ref, m_ref):
        k = kvbuf[0, slot_of(t), p]
        s = lax.dot_general(q, k, _NT, preferred_element_type=jnp.float32)
        s_ref[...] = s
        m_ref[...] = jnp.broadcast_to(jnp.max(s, axis=-1, keepdims=True), m_ref.shape)

    def stage_C(s_ref, m_ref, p_ref, r_ref):
        m = m_ref[...]
        n = s_ref.shape[1] // 128
        lsum = None
        for c in range(n):
            pc = jnp.exp2(s_ref[:, c * 128:(c + 1) * 128] - m)
            lsum = pc if lsum is None else lsum + pc
            p_ref[:, c * 128:(c + 1) * 128] = pltpu.bitcast(pc.astype(jnp.bfloat16), jnp.uint32)
        l = jnp.sum(lsum, axis=-1, keepdims=True)
        r_ref[...] = jnp.broadcast_to(1.0 / l, r_ref.shape)

    def stage_D(t, p, p_ref, r_ref):
        v = kvbuf[1, slot_of(t), p]
        pp = pltpu.bitcast(p_ref[...], jnp.bfloat16)
        o = jnp.dot(pp, v, preferred_element_type=jnp.float32)
        return (o * r_ref[...]).astype(jnp.bfloat16)

    def stage_E(t, p, o):
        b, h = bh(t, p)
        c0 = pl.multiple_of(h * 128, 128)
        acc[t & 1, :, p * D:(p + 1) * D] += jnp.dot(o, wobuf[p, pl.ds(c0, 128), :], preferred_element_type=jnp.float32)

    NBATCH = out_hbm.shape[0]

    def out_copy(b):
        return pltpu.make_async_copy(obuf.at[b], out_hbm.at[b], osem.at[b])

    def flush_out(t, last):
        b, h = bh(t)
        g = t & 1
        obuf[b] = acc[g].astype(obuf.dtype)
        if last:
            out_copy(b).start()
        else:
            acc[g] = jnp.zeros(acc.shape[1:], acc.dtype)
            rnd = t >> (hshift + 1)
            @pl.when(jnp.logical_or(rnd < NEARLY, rnd == NBATCH // 2 - 1))
            def _():
                out_copy(b).start()

    def body(t, doAB, doDE, do_issue):
        if NO_COMPUTE:
            doAB = doDE = False
        pts = iter(range(NPC))
        def pt():
            if do_issue:
                for _ in range(GRP):
                    i = next(pts, None)
                    if i is not None:
                        issue(i, t)
        pt()
        if doAB:
            qa = stage_A(t, 0)
            qb = stage_A(t, 1)
        pt()
        if doDE:
            stage_C(s1, m1, p1, r1)
            pt()
            o0 = stage_D(t - 1, 0, p0, r0)
        pt()
        if doAB:
            stage_B(qa, t, 0, s0, m0)
        pt()
        if doDE:
            o1 = stage_D(t - 1, 1, p1, r1)
        pt()
        if doAB:
            stage_C(s0, m0, p0, r0)
            pt()
            stage_B(qb, t, 1, s1, m1)
        pt()
        if doDE:
            stage_E(t - 1, 0, o0)
            stage_E(t - 1, 1, o1)
        for _ in range(NPC):
            pt()

    HD = wqbuf.shape[-1]
    QC = HD // 2
    OR = 32
    nwp = (D // 8) * 2
    assert nwp == HD // OR
    XR = 32
    nxp = xbuf.shape[1] * xbuf.shape[2] // XR
    xpb = xbuf.shape[2] // XR

    def wloop(i, c):
        r8 = pl.multiple_of((i >> 1) * 8, 8)
        c0 = pl.multiple_of((i & 1) * QC, QC)
        r32 = pl.multiple_of(i * OR, OR)
        for p, (wq, wo) in enumerate(((wqa, woa), (wqb, wob))):
            pltpu.make_async_copy(wq.at[pl.ds(r8, 8), pl.ds(c0, QC)], wqbuf.at[p, pl.ds(r8, 8), pl.ds(c0, QC)],
                                  wsem.at[1 + 2 * p]).start(priority=WPRIO[2 * p])
            pltpu.make_async_copy(wo.at[pl.ds(r32, OR)], wobuf.at[p, pl.ds(r32, OR)],
                                  wsem.at[4 + p]).start(priority=WPRIO[2 * p + 1])
        return c

    def xloop(i, c):
        b = i // xpb
        r = pl.multiple_of((i % xpb) * XR, XR)
        for p, x in enumerate((xa, xb)):
            pltpu.make_async_copy(x.at[b, pl.ds(r, XR)], xbuf.at[p, b, pl.ds(r, XR)], wsem.at[2 * p]).start(priority=p)
        return c

    lax.fori_loop(0, nxp, xloop, 0)
    lax.fori_loop(0, nwp, wloop, 0)
    for need in range(L):
        for pc in range(NPC):
            for s in range(4):
                start_piece(s, need, pc * PIECE, PRIO[s])
    acc[...] = jnp.zeros_like(acc)
    for c in w_copies[:4]:
        c.wait()
    wait_kv(0, 0)
    body(jnp.int32(0), True, False, True)
    for c in w_copies[4:]:
        c.wait()

    def loop(t, carry):
        wait_kv(0, t)
        wait_kv(1, t - 1)
        body(t, True, True, True)
        @pl.when((((t - 1) >> 1) & (n_heads - 1)) == n_heads - 1)
        def _():
            flush_out(t - 1, False)
        deferred = [b for rnd in range(NEARLY, NBATCH // 2 - 1) for b in (rnd, rnd + NBATCH // 2)]
        for td in sorted(set(TDEF)):
            @pl.when(t == N - td)
            def _():
                for b, d in zip(deferred, TDEF):
                    if d == td:
                        out_copy(b).start(priority=OPRIO)
        return carry

    lax.fori_loop(1, N, loop, 0)

    wait_kv(1, N - 1)
    body(N, False, True, False)
    flush_out(N - 1, True)
    for b in range(NBATCH):
        out_copy(b).wait()


@jax.jit
def pallas_concat_heads__mha_block_cached__gqa_block_cached__near_ridge_kernel(
    A_x, A_k_cache, A_v_cache, A_wq, A_wo, B_x, B_k_cache, B_v_cache, B_wq, B_wo):
    B, Sq, D = A_x.shape
    _, H, Sk, Dh = A_k_cache.shape
    n = B * H
    r = lambda a: a.reshape(n, Sk, Dh)
    qscale = (Dh ** -0.5) * math.log2(math.e)
    kern = functools.partial(_kernel, n_units=n, n_heads=H, qscale=qscale)
    bf = jnp.bfloat16
    f32 = jnp.float32
    u32 = jnp.uint32
    ps = pltpu.VMEM((Sq // 2, Sk), u32)
    return pl.pallas_call(
        kern,
        in_specs=[pl.BlockSpec(memory_space=pl.ANY)] * 10,
        out_specs=pl.BlockSpec(memory_space=pl.ANY),
        out_shape=jax.ShapeDtypeStruct((B, Sq, 2 * D), A_x.dtype),
        scratch_shapes=[
            pltpu.VMEM((2, B, Sq, D), bf),
            pltpu.VMEM((2, D, H * Dh), bf),
            pltpu.VMEM((2, H * Dh, D), bf),
            pltpu.VMEM((2, NB, 2, Sk, Dh), bf),
            pltpu.VMEM((Sq, Sk), f32), pltpu.VMEM((Sq, Sk), f32),
            pltpu.VMEM((Sq, 128), f32), pltpu.VMEM((Sq, 128), f32),
            ps, ps,
            pltpu.VMEM((Sq, 128), f32), pltpu.VMEM((Sq, 128), f32),
            pltpu.VMEM((2, Sq, 2 * D), f32),
            pltpu.VMEM((B, Sq, 2 * D), bf),
            pltpu.SemaphoreType.DMA((6,)),
            pltpu.SemaphoreType.DMA((2, NB)),
            pltpu.SemaphoreType.DMA((B,)),
        ],
        compiler_params=pltpu.CompilerParams(vmem_limit_bytes=100 * 1024 * 1024, disable_bounds_checks=True),
    )(A_x, r(A_k_cache), r(A_v_cache), A_wq, A_wo, B_x, r(B_k_cache), r(B_v_cache), B_wq, B_wo)
```

```python
import functools
import math

import jax
import jax.numpy as jnp
from jax import lax
import jax.experimental.pallas as pl
import jax.experimental.pallas.tpu as pltpu

NB = 8
G = 2
L = 3
PIECE = 64
PRIO = (1, 1, 1, 0)
WPRIO = (0, 1, 1, 1)
NPT = 8
TDEF = 3
TSWITCH = 8

_NT = (((1,), (1,)), ((), ()))


def _kernel(xa, ka, va, wqa, woa, xb, kb, vb, wqb, wob, out_hbm,
            xbuf, wqbuf, wobuf, kvbuf, s0, s1, m0, m1, p0, p1, r0, r1, acc, obuf,
            wsem, kvsem, osem, *, n_heads, qscale):
    N, Sk, Dh = ka.shape
    _, NBATCH, Sq, D = xbuf.shape
    HD = wqbuf.shape[-1]
    hshift = n_heads.bit_length() - 1
    gshift = G.bit_length() - 1
    NPC = Sk // PIECE
    NRND = NBATCH // G
    assert n_heads == 1 << hshift and NBATCH % G == 0
    assert G <= L <= NB - G and TSWITCH % G == 0 and NPC % NPT == 0 and NPC % G == 0

    srcs = (ka, va, kb, vb)

    def slot_of(t):
        return t & (NB - 1)

    def unit_of(t):
        g, j = t & (G - 1), t >> gshift
        return g * (N // G) + (j & ~(n_heads - 1)) + ((j + g * (n_heads // 2)) & (n_heads - 1))

    def bh(t):
        u = unit_of(t)
        return u >> hshift, u & (n_heads - 1)

    def piece_copy(s, t, off):
        slot = slot_of(t)
        off = pl.multiple_of(off, PIECE)
        return pltpu.make_async_copy(
            srcs[s].at[unit_of(t), pl.ds(off, PIECE)],
            kvbuf.at[s % 2, slot, s // 2, pl.ds(off, PIECE)],
            kvsem.at[s % 2, slot])

    def start_pieces(need, off, head=False):
        for s in range(4):
            t = need - (s % 2)

            @pl.when(t >= 0 if head else t < N)
            def _():
                piece_copy(s, t, off).start(priority=PRIO[s])

    def issue(i, t):
        inter = t < N - TSWITCH
        need = jnp.where(inter, (t & ~(G - 1)) + L + i % G, t + L)
        off = jnp.where(inter, (t & (G - 1)) * (Sk // G) + (i // G) * PIECE, i * PIECE)
        start_pieces(need, off)

    def wait_kv(which, t):
        slot = slot_of(t)
        pltpu.make_async_copy(kvbuf.at[which, slot], kvbuf.at[which, slot], kvsem.at[which, slot]).wait()

    def stage_A(t, p):
        b, h = bh(t)
        c0 = pl.multiple_of(h * Dh, Dh)
        q = jnp.dot(xbuf[p, b], wqbuf[p, :, pl.ds(c0, Dh)], preferred_element_type=jnp.float32)
        return (q * qscale).astype(jnp.bfloat16)

    def stage_B(q, t, p, s_ref, m_ref):
        k = kvbuf[0, slot_of(t), p]
        s = lax.dot_general(q, k, _NT, preferred_element_type=jnp.float32)
        s_ref[...] = s
        m_ref[...] = jnp.broadcast_to(jnp.max(s, axis=-1, keepdims=True), m_ref.shape)

    def stage_C(s_ref, m_ref, p_ref, r_ref):
        m = m_ref[...]
        lsum = None
        for c in range(Sk // 128):
            pc = jnp.exp2(s_ref[:, c * 128:(c + 1) * 128] - m)
            lsum = pc if lsum is None else lsum + pc
            p_ref[:, c * 128:(c + 1) * 128] = pltpu.bitcast(pc.astype(jnp.bfloat16), jnp.uint32)
        l = jnp.sum(lsum, axis=-1, keepdims=True)
        r_ref[...] = jnp.broadcast_to(1.0 / l, r_ref.shape)

    def stage_D(t, p, p_ref, r_ref):
        v = kvbuf[1, slot_of(t), p]
        pp = pltpu.bitcast(p_ref[...], jnp.bfloat16)
        o = jnp.dot(pp, v, preferred_element_type=jnp.float32)
        return (o * r_ref[...]).astype(jnp.bfloat16)

    def stage_E(t, p, o):
        _, h = bh(t)
        c0 = pl.multiple_of(h * Dh, Dh)
        acc[t & (G - 1), :, p * D:(p + 1) * D] += jnp.dot(
            o, wobuf[p, pl.ds(c0, Dh), :], preferred_element_type=jnp.float32)

    def body(t, do_ab, do_de, do_issue):
        groups = iter(range(NPC))

        def pt():
            if do_issue:
                for _ in range(NPC // NPT):
                    i = next(groups, None)
                    if i is not None:
                        issue(i, t)

        pt()
        if do_ab:
            qa = stage_A(t, 0)
            qb = stage_A(t, 1)
        pt()
        if do_de:
            stage_C(s1, m1, p1, r1)
            pt()
            o0 = stage_D(t - 1, 0, p0, r0)
        pt()
        if do_ab:
            stage_B(qa, t, 0, s0, m0)
        pt()
        if do_de:
            o1 = stage_D(t - 1, 1, p1, r1)
        pt()
        if do_ab:
            stage_C(s0, m0, p0, r0)
            pt()
            stage_B(qb, t, 1, s1, m1)
        pt()
        if do_de:
            stage_E(t - 1, 0, o0)
            stage_E(t - 1, 1, o1)
        for _ in range(NPT):
            pt()

    def out_copy(b):
        return pltpu.make_async_copy(obuf.at[b], out_hbm.at[b], osem.at[b])

    def flush_out(t, last):
        b, _ = bh(t)
        g = t & (G - 1)
        obuf[b] = acc[g].astype(obuf.dtype)
        if last:
            out_copy(b).start()
        else:
            acc[g] = jnp.zeros(acc.shape[1:], acc.dtype)

            @pl.when(t >= N - TDEF)
            def _():
                out_copy(b).start()

    nwp = (D // 8) * 2
    QC = HD // 2
    OR = HD // nwp
    XR = 32
    xpb = Sq // XR

    def xloop(i, c):
        b = i // xpb
        r = pl.multiple_of((i % xpb) * XR, XR)
        for p, x in enumerate((xa, xb)):
            pltpu.make_async_copy(x.at[b, pl.ds(r, XR)], xbuf.at[p, b, pl.ds(r, XR)],
                                  wsem.at[0, p]).start(priority=p)
        return c

    def wloop(i, c):
        r8 = pl.multiple_of((i >> 1) * 8, 8)
        c0 = pl.multiple_of((i & 1) * QC, QC)
        ro = pl.multiple_of(i * OR, OR)
        for p, (wq, wo) in enumerate(((wqa, woa), (wqb, wob))):
            pltpu.make_async_copy(wq.at[pl.ds(r8, 8), pl.ds(c0, QC)],
                                  wqbuf.at[p, pl.ds(r8, 8), pl.ds(c0, QC)],
                                  wsem.at[1, p]).start(priority=WPRIO[2 * p])
            pltpu.make_async_copy(wo.at[pl.ds(ro, OR)], wobuf.at[p, pl.ds(ro, OR)],
                                  wsem.at[2, p]).start(priority=WPRIO[2 * p + 1])
        return c

    def kv0loop(i, c):
        start_pieces(i // NPC, (i % NPC) * PIECE, head=True)
        return c

    def wait_w(k, buf):
        for p in range(2):
            pltpu.make_async_copy(buf.at[p], buf.at[p], wsem.at[k, p]).wait()

    lax.fori_loop(0, NBATCH * xpb, xloop, 0)
    lax.fori_loop(0, nwp, wloop, 0)
    lax.fori_loop(0, L * NPC, kv0loop, 0)
    acc[...] = jnp.zeros_like(acc)
    wait_w(0, xbuf)
    wait_w(1, wqbuf)
    wait_kv(0, 0)
    body(jnp.int32(0), True, False, True)
    wait_w(2, wobuf)

    def loop(t, carry):
        wait_kv(0, t)
        wait_kv(1, t - 1)
        body(t, True, True, True)

        @pl.when((((t - 1) >> gshift) & (n_heads - 1)) == n_heads - 1)
        def _():
            flush_out(t - 1, False)

        @pl.when(t == N - TDEF)
        def _():
            for b in range(NBATCH):
                g, rnd = b // NRND, b % NRND
                if ((rnd + 1) * n_heads - 1) * G + g < N - TDEF:
                    out_copy(b).start()

        return carry

    lax.fori_loop(1, N, loop, 0)

    wait_kv(1, N - 1)
    body(N, False, True, False)
    flush_out(N - 1, True)
    for b in range(NBATCH):
        out_copy(b).wait()


@jax.jit
def pallas_concat_heads__mha_block_cached__gqa_block_cached__near_ridge_kernel(
    A_x: jax.Array,
    A_k_cache: jax.Array,
    A_v_cache: jax.Array,
    A_wq: jax.Array,
    A_wo: jax.Array,
    B_x: jax.Array,
    B_k_cache: jax.Array,
    B_v_cache: jax.Array,
    B_wq: jax.Array,
    B_wo: jax.Array,
):
    B, Sq, D = A_x.shape
    _, H, Sk, Dh = A_k_cache.shape
    assert B_k_cache.shape == A_k_cache.shape and A_wq.shape == B_wq.shape == (D, H * Dh)
    flat = lambda a: a.reshape(B * H, Sk, Dh)
    kern = functools.partial(_kernel, n_heads=H, qscale=(Dh ** -0.5) * math.log2(math.e))
    bf, f32, u32 = jnp.bfloat16, jnp.float32, jnp.uint32
    return pl.pallas_call(
        kern,
        in_specs=[pl.BlockSpec(memory_space=pl.ANY)] * 10,
        out_specs=pl.BlockSpec(memory_space=pl.ANY),
        out_shape=jax.ShapeDtypeStruct((B, Sq, 2 * D), A_x.dtype),
        scratch_shapes=[
            pltpu.VMEM((2, B, Sq, D), bf),
            pltpu.VMEM((2, D, H * Dh), bf),
            pltpu.VMEM((2, H * Dh, D), bf),
            pltpu.VMEM((2, NB, 2, Sk, Dh), bf),
            pltpu.VMEM((Sq, Sk), f32), pltpu.VMEM((Sq, Sk), f32),
            pltpu.VMEM((Sq, 128), f32), pltpu.VMEM((Sq, 128), f32),
            pltpu.VMEM((Sq // 2, Sk), u32), pltpu.VMEM((Sq // 2, Sk), u32),
            pltpu.VMEM((Sq, 128), f32), pltpu.VMEM((Sq, 128), f32),
            pltpu.VMEM((G, Sq, 2 * D), f32),
            pltpu.VMEM((B, Sq, 2 * D), bf),
            pltpu.SemaphoreType.DMA((3, 2)),
            pltpu.SemaphoreType.DMA((2, NB)),
            pltpu.SemaphoreType.DMA((B,)),
        ],
        compiler_params=pltpu.CompilerParams(
            vmem_limit_bytes=100 * 1024 * 1024, disable_bounds_checks=True),
    )(A_x, flat(A_k_cache), flat(A_v_cache), A_wq, A_wo,
      B_x, flat(B_k_cache), flat(B_v_cache), B_wq, B_wo)
```

```python
import functools
import math

import jax
import jax.numpy as jnp
from jax import lax
import jax.experimental.pallas as pl
import jax.experimental.pallas.tpu as pltpu

NB = 8
G = 2
L = 3
PIECE = 64
PRIO = (1, 1, 1, 0)
WPRIO = (0, 1, 1, 1)
WQS = 4
WH = 2
NPT = 8
TDEF = 3
TSWITCH = 8

_NT = (((1,), (1,)), ((), ()))


def _kernel(xa, ka, va, wqa, woa, xb, kb, vb, wqb, wob, out_hbm,
            xbuf, wqbuf, wobuf, kvbuf, s0, s1, m0, m1, p0, p1, r0, r1, acc, obuf,
            wsem, kvsem, osem, *, n_heads, qscale):
    N, Sk, Dh = ka.shape
    _, NBATCH, Sq, D = xbuf.shape
    HD = wqbuf.shape[-1]
    hshift = n_heads.bit_length() - 1
    gshift = G.bit_length() - 1
    NPC = Sk // PIECE
    NRND = NBATCH // G
    assert n_heads == 1 << hshift and NBATCH % G == 0
    assert G <= L <= NB - G and TSWITCH % G == 0 and NPC % NPT == 0 and NPC % G == 0

    srcs = (ka, va, kb, vb)

    def slot_of(t):
        return t & (NB - 1)

    def unit_of(t):
        g, j = t & (G - 1), t >> gshift
        return g * (N // G) + (j & ~(n_heads - 1)) + ((j + g * (n_heads // 2)) & (n_heads - 1))

    def bh(t):
        u = unit_of(t)
        return u >> hshift, u & (n_heads - 1)

    def piece_copy(s, t, off):
        slot = slot_of(t)
        off = pl.multiple_of(off, PIECE)
        return pltpu.make_async_copy(
            srcs[s].at[unit_of(t), pl.ds(off, PIECE)],
            kvbuf.at[s % 2, slot, s // 2, pl.ds(off, PIECE)],
            kvsem.at[s % 2, slot])

    def start_pieces(need, off, head=False):
        for s in range(4):
            t = need - (s % 2)

            @pl.when(t >= 0 if head else t < N)
            def _():
                piece_copy(s, t, off).start(priority=PRIO[s])

    def issue(i, t):
        inter = t < N - TSWITCH
        need = jnp.where(inter, (t & ~(G - 1)) + L + i % G, t + L)
        off = jnp.where(inter, (t & (G - 1)) * (Sk // G) + (i // G) * PIECE, i * PIECE)
        start_pieces(need, off)

    def wait_kv(which, t):
        slot = slot_of(t)
        pltpu.make_async_copy(kvbuf.at[which, slot], kvbuf.at[which, slot], kvsem.at[which, slot]).wait()

    def stage_A(t, p):
        b, h = bh(t)
        c0 = pl.multiple_of(h * Dh, Dh)
        q = jnp.dot(xbuf[p, b], wqbuf[p, :, pl.ds(c0, Dh)], preferred_element_type=jnp.float32)
        return q.astype(jnp.bfloat16)

    def stage_B(q, t, p, s_ref, m_ref):
        k = kvbuf[0, slot_of(t), p]
        s = lax.dot_general(q, k, _NT, preferred_element_type=jnp.float32)
        s_ref[...] = s
        m_ref[...] = jnp.broadcast_to(jnp.max(s, axis=-1, keepdims=True), m_ref.shape)

    def stage_C(s_ref, m_ref, p_ref, r_ref):
        m = m_ref[...]
        lsum = None
        for c in range(Sk // 128):
            pc = jnp.exp2((s_ref[:, c * 128:(c + 1) * 128] - m) * qscale)
            lsum = pc if lsum is None else lsum + pc
            p_ref[:, c * 128:(c + 1) * 128] = pltpu.bitcast(pc.astype(jnp.bfloat16), jnp.uint32)
        l = jnp.sum(lsum, axis=-1, keepdims=True)
        r_ref[...] = jnp.broadcast_to(1.0 / l, r_ref.shape)

    def stage_D(t, p, p_ref, r_ref):
        v = kvbuf[1, slot_of(t), p]
        pp = pltpu.bitcast(p_ref[...], jnp.bfloat16)
        o = jnp.dot(pp, v, preferred_element_type=jnp.float32)
        return (o * r_ref[...]).astype(jnp.bfloat16)

    def stage_E(t, p, o):
        _, h = bh(t)
        c0 = pl.multiple_of(h * Dh, Dh)
        acc[t & (G - 1), :, p * D:(p + 1) * D] += jnp.dot(
            o, wobuf[p, pl.ds(c0, Dh), :], preferred_element_type=jnp.float32)

    def body(t, do_ab, do_de, do_issue):
        groups = iter(range(NPC))

        def pt():
            if do_issue:
                for _ in range(NPC // NPT):
                    i = next(groups, None)
                    if i is not None:
                        issue(i, t)

        pt()
        if do_ab:
            qa = stage_A(t, 0)
            qb = stage_A(t, 1)
        pt()
        if do_de:
            stage_C(s1, m1, p1, r1)
            pt()
            o0 = stage_D(t - 1, 0, p0, r0)
        pt()
        if do_ab:
            stage_B(qa, t, 0, s0, m0)
        pt()
        if do_de:
            o1 = stage_D(t - 1, 1, p1, r1)
        pt()
        if do_ab:
            stage_C(s0, m0, p0, r0)
            pt()
            stage_B(qb, t, 1, s1, m1)
        pt()
        if do_de:
            stage_E(t - 1, 0, o0)
            stage_E(t - 1, 1, o1)
        for _ in range(NPT):
            pt()

    def out_copy(b):
        return pltpu.make_async_copy(obuf.at[b], out_hbm.at[b], osem.at[b])

    def flush_out(t, last):
        b, _ = bh(t)
        g = t & (G - 1)
        obuf[b] = acc[g].astype(obuf.dtype)
        if last:
            out_copy(b).start()
        else:
            acc[g] = jnp.zeros(acc.shape[1:], acc.dtype)

            @pl.when(t >= N - TDEF)
            def _():
                out_copy(b).start()

    nwp = (D // 8) * WQS
    QC = HD // WQS
    OR = HD // nwp
    XR = 32
    xpb = Sq // XR

    def xloop(i, c):
        b = i // xpb
        r = pl.multiple_of((i % xpb) * XR, XR)
        for p, x in enumerate((xa, xb)):
            pltpu.make_async_copy(x.at[b, pl.ds(r, XR)], xbuf.at[p, b, pl.ds(r, XR)],
                                  wsem.at[0, p]).start(priority=p)
        return c

    def wloop(i0, c):
        for hf in range(WH):
            i = i0 + hf * (nwp // WH)
            r8 = pl.multiple_of((i // WQS) * 8, 8)
            c0 = pl.multiple_of((i % WQS) * QC, QC)
            ro = pl.multiple_of(i * OR, OR)
            for p, (wq, wo) in enumerate(((wqa, woa), (wqb, wob))):
                pltpu.make_async_copy(wq.at[pl.ds(r8, 8), pl.ds(c0, QC)],
                                      wqbuf.at[p, pl.ds(r8, 8), pl.ds(c0, QC)],
                                      wsem.at[1, p]).start(priority=WPRIO[2 * p])
                pltpu.make_async_copy(wo.at[pl.ds(ro, OR)], wobuf.at[p, pl.ds(ro, OR)],
                                      wsem.at[2, p]).start(priority=WPRIO[2 * p + 1])
        return c

    def kv0loop(i, c):
        start_pieces(i // NPC, (i % NPC) * PIECE, head=True)
        return c

    def wait_w(k, buf):
        for p in range(2):
            pltpu.make_async_copy(buf.at[p], buf.at[p], wsem.at[k, p]).wait()

    lax.fori_loop(0, NBATCH * xpb, xloop, 0)
    lax.fori_loop(0, nwp // WH, wloop, 0)
    lax.fori_loop(0, L * NPC, kv0loop, 0)
    acc[...] = jnp.zeros_like(acc)
    wait_w(0, xbuf)
    wait_w(1, wqbuf)
    wait_kv(0, 0)
    body(jnp.int32(0), True, False, True)
    wait_w(2, wobuf)

    def loop(t, carry):
        wait_kv(0, t)
        wait_kv(1, t - 1)
        body(t, True, True, True)

        @pl.when((((t - 1) >> gshift) & (n_heads - 1)) == n_heads - 1)
        def _():
            flush_out(t - 1, False)

        @pl.when(t == N - TDEF)
        def _():
            for b in range(NBATCH):
                g, rnd = b // NRND, b % NRND
                if ((rnd + 1) * n_heads - 1) * G + g < N - TDEF:
                    out_copy(b).start()

        return carry

    lax.fori_loop(1, N, loop, 0)

    wait_kv(1, N - 1)
    body(N, False, True, False)
    flush_out(N - 1, True)
    for b in range(NBATCH):
        out_copy(b).wait()


@jax.jit
def pallas_concat_heads__mha_block_cached__gqa_block_cached__near_ridge_kernel(
    A_x: jax.Array,
    A_k_cache: jax.Array,
    A_v_cache: jax.Array,
    A_wq: jax.Array,
    A_wo: jax.Array,
    B_x: jax.Array,
    B_k_cache: jax.Array,
    B_v_cache: jax.Array,
    B_wq: jax.Array,
    B_wo: jax.Array,
):
    B, Sq, D = A_x.shape
    _, H, Sk, Dh = A_k_cache.shape
    assert B_k_cache.shape == A_k_cache.shape and A_wq.shape == B_wq.shape == (D, H * Dh)
    flat = lambda a: a.reshape(B * H, Sk, Dh)
    kern = functools.partial(_kernel, n_heads=H, qscale=(Dh ** -0.5) * math.log2(math.e))
    bf, f32, u32 = jnp.bfloat16, jnp.float32, jnp.uint32
    return pl.pallas_call(
        kern,
        in_specs=[pl.BlockSpec(memory_space=pl.ANY)] * 10,
        out_specs=pl.BlockSpec(memory_space=pl.ANY),
        out_shape=jax.ShapeDtypeStruct((B, Sq, 2 * D), A_x.dtype),
        scratch_shapes=[
            pltpu.VMEM((2, B, Sq, D), bf),
            pltpu.VMEM((2, D, H * Dh), bf),
            pltpu.VMEM((2, H * Dh, D), bf),
            pltpu.VMEM((2, NB, 2, Sk, Dh), bf),
            pltpu.VMEM((Sq, Sk), f32), pltpu.VMEM((Sq, Sk), f32),
            pltpu.VMEM((Sq, 128), f32), pltpu.VMEM((Sq, 128), f32),
            pltpu.VMEM((Sq // 2, Sk), u32), pltpu.VMEM((Sq // 2, Sk), u32),
            pltpu.VMEM((Sq, 128), f32), pltpu.VMEM((Sq, 128), f32),
            pltpu.VMEM((G, Sq, 2 * D), f32),
            pltpu.VMEM((B, Sq, 2 * D), bf),
            pltpu.SemaphoreType.DMA((3, 2)),
            pltpu.SemaphoreType.DMA((2, NB)),
            pltpu.SemaphoreType.DMA((B,)),
        ],
        compiler_params=pltpu.CompilerParams(
            vmem_limit_bytes=100 * 1024 * 1024, disable_bounds_checks=True),
    )(A_x, flat(A_k_cache), flat(A_v_cache), A_wq, A_wo,
      B_x, flat(B_k_cache), flat(B_v_cache), B_wq, B_wo)
```
